```python
import os as _os
_os.environ.setdefault("JAX_PLATFORMS", "cpu")
import jax
import jax.numpy as jnp

def _softmax(x, axis=-1):
    return jax.nn.softmax(x, axis=axis)
def _gelu(x):
    return jax.nn.gelu(x, approximate=True)
def _silu(x):
    return jax.nn.silu(x)
def _sigmoid(x):
    return jax.nn.sigmoid(x)
def _layernorm(x, axis=-1, eps=1e-5):
    m = jnp.mean(x, axis=axis, keepdims=True)
    v = jnp.var(x, axis=axis, keepdims=True)
    return (x - m) / jnp.sqrt(v + eps)
def _scatter_add(tgt, idx, src, axis=0):
    return tgt.at[idx].add(src)
def _segment_sum(src, seg, n):
    return jax.ops.segment_sum(src, seg, n)
class _Rng:
    def __init__(self, key):
        self._k = key
    def _next(self):
        self._k, sub = jax.random.split(self._k)
        return sub
    def normal(self, shape):
        return jax.random.normal(self._next(), shape, dtype=jnp.bfloat16)
    def randint(self, lo, hi, shape):
        return jax.random.randint(self._next(), shape, lo, hi, dtype=jnp.int32)
    def uniform(self, shape, lo=0.0, hi=1.0):
        return jax.random.uniform(self._next(), shape, jnp.bfloat16, lo, hi)
    def permutation(self, n):
        return jax.random.permutation(self._next(), n)


kernel_name = 'sequential_preLN__compressed_kv_cla__dense_activation_mish__decode'

def setup_inputs():
    _rng = _Rng(jax.random.key(int.from_bytes(__import__("os").urandom(4), "little")))
    _w = (lambda a: (lambda t: t.astype(jnp.bfloat16) if jnp.issubdtype(t.dtype, jnp.floating) else t)(jnp.asarray(a)))
    def _A_setup():
        B, H, Sq, Sk, D, M = 1, 32, 1, 8192, 128, 512
        Dc = 4 * D
        return {
            "x": _w((lambda *s: _rng.normal(s) * 0.05)(B, Sq, M)),
            "c_kv": _w((lambda *s: _rng.normal(s) * 0.8)(B, Sk, Dc)),
            "w_q": _w((lambda *s: _rng.normal(s) * 0.8)(M, H, D) * (M ** -0.5)),
            "w_uk": _w((lambda *s: _rng.normal(s) * 0.8)(Dc, H, D) * (Dc ** -0.5)),
            "w_uv": _w((lambda *s: _rng.normal(s) * 0.8)(Dc, H, D) * (Dc ** -0.5)),
            "w_o": _w((lambda *s: _rng.normal(s) * 0.8)(H, D, M) * ((H * D) ** -0.5)),
        }
    _A_in = _A_setup()

    def _B_setup():
        B, S, D, F = 1, 1, 512, 1376
        return {
            "x": _w((lambda *s: _rng.normal(s) * 0.05)(B, S, D)),
            "w1": _w((lambda *s: _rng.normal(s) * 0.2)(D, F) * (D ** -0.5)),
            "b1": _w((lambda *s: _rng.normal(s) * 0.05)(F)),
            "w2": _w((lambda *s: _rng.normal(s) * 0.05)(F, D) * (F ** -0.5)),
        }
    _B_in = _B_setup()

    return {
        "A_x": _A_in["x"],
        "A_c_kv": _A_in["c_kv"],
        "A_w_q": _A_in["w_q"],
        "A_w_uk": _A_in["w_uk"],
        "A_w_uv": _A_in["w_uv"],
        "A_w_o": _A_in["w_o"],
        "B_x": _B_in["x"],
        "B_w1": _B_in["w1"],
        "B_b1": _B_in["b1"],
        "B_w2": _B_in["w2"],
    }

def reference(A_x, A_c_kv, A_w_q, A_w_uk, A_w_uv, A_w_o, B_x, B_w1, B_b1, B_w2):
    def _A_ref(x, c_kv, w_q, w_uk, w_uv, w_o):
        B, Sq, M = x.shape[0], x.shape[1], x.shape[2]
        Sk = c_kv.shape[1]
        H, D = w_q.shape[1], w_q.shape[2]
        q = jnp.einsum("bqm,mhd->bhqd", x, w_q)
        k = jnp.einsum("bkc,chd->bhkd", c_kv, w_uk)
        v = jnp.einsum("bkc,chd->bhkd", c_kv, w_uv)
        scores = jnp.einsum("bhqd,bhkd->bhqk", q, k) * (D ** -0.5)
        off = Sk - Sq
        qi = jnp.arange(Sq)[:, None]
        kj = jnp.arange(Sk)[None, :]
        cmask = kj <= (qi + off)
        scores = jnp.where(cmask[None, None], scores, -1e9)
        p = _softmax(scores, axis=-1)
        ctx = jnp.einsum("bhqk,bhkd->bhqd", p, v)
        return jnp.einsum("bhqd,hdm->bqm", ctx, w_o)

    def _B_ref(x, w1, b1, w2):
        h = jnp.einsum("bsd,df->bsf", x, w1) + b1
        sp = jnp.log1p(jnp.exp(-jnp.abs(h))) + jnp.where(h > 0, h, jnp.zeros_like(h))
        act = h * jnp.tanh(sp)
        return jnp.einsum("bsf,fd->bsd", act, w2)

    x = A_x
    h = x + _A_ref(_layernorm(x, axis=-1), A_c_kv, A_w_q, A_w_uk, A_w_uv, A_w_o)
    h2 = h + _B_ref(_layernorm(h, axis=-1), B_w1, B_b1, B_w2)
    return h2
```

```python
import functools
import jax
import jax.numpy as jnp
import jax.experimental.pallas as pl
import jax.experimental.pallas.tpu as pltpu
from jax import lax

F32 = jnp.float32
BF16 = jnp.bfloat16

H, D, M, SK, DC, F = 32, 128, 512, 8192, 512, 1376

def _ln(v):
    m = jnp.mean(v, axis=-1, keepdims=True)
    c = v - m
    var = jnp.mean(c * c, axis=-1, keepdims=True)
    return c / jnp.sqrt(var + 1e-5)

def build(nq=4, nkv=16, no=4, window=3, f_chunks=((0, 512), (512, 512), (1024, 352)), f2_chunks=None):
    cq = 16384 // nq
    bk = SK // nkv
    co = 4096 // no
    f1 = list(f_chunks)
    f2 = list(f2_chunks) if f2_chunks else list(f_chunks)

    def kernel(x_hbm, ckv_hbm, wq_hbm, wuk_hbm, wuv_hbm, wo_hbm, w1_hbm, b1_hbm, w2_hbm, o_ref,
               xb, b1b, qb, ukb, cb, uvb, ob, w1b, w2b, sem_s, sem_q, sem_uk, sem_c, sem_uv, sem_o, sem_1, sem_2):
        plan = []
        base = {}
        def add(name, src, dst, sem, chunks):
            base[name] = len(plan)
            for i, (s, n) in enumerate(chunks): plan.append((src, dst, sem, i, s, n))
        add('q', wq_hbm, qb, sem_q, [(i*cq, cq) for i in range(nq)])
        add('uk', wuk_hbm, ukb, sem_uk, [(i*cq, cq) for i in range(nq)])
        add('c', ckv_hbm, cb, sem_c, [(i*bk, bk) for i in range(nkv)])
        add('uv', wuv_hbm, uvb, sem_uv, [(i*cq, cq) for i in range(nq)])
        add('o', wo_hbm, ob, sem_o, [(i*co, co) for i in range(no)])
        add('w1', w1_hbm, w1b, sem_1, f1)
        add('w2', w2_hbm, w2b, sem_2, f2)
        NP = len(plan)
        def cp(j):
            src, dst, sem, i, s, n = plan[j]
            return pltpu.make_async_copy(src.at[pl.ds(s, n)], dst.at[pl.ds(s, n)], sem.at[i])
        W = window
        def wait(name, i):
            j = base[name] + i
            cp(j).wait()
            if j + W < NP: cp(j + W).start()
        cx = pltpu.make_async_copy(x_hbm, xb, sem_s.at[0])
        cb1 = pltpu.make_async_copy(b1_hbm, b1b, sem_s.at[1])
        cp(0).start()
        cx.start()
        for j in range(1, min(W, NP)): cp(j).start()
        cb1.start()

        cx.wait()
        x = xb[...].astype(F32)
        xn = _ln(x).astype(BF16).astype(F32)

        row = lax.broadcasted_iota(jnp.int32, (H, 128), 0)
        lane = lax.broadcasted_iota(jnp.int32, (H, 128), 1)
        diag = (lane % 32) == row
        lane_grp = lane // 32
        tiles_per_chunk = cq // 128

        def contract_lead(a, wref, name):
            acc = jnp.zeros((H, D), F32)
            for ch in range(nq):
                wait(name, ch)
                ls = []
                for tt in range(tiles_per_chunk):
                    t = ch * tiles_per_chunk + tt
                    k, s = t // 32, t % 32
                    ak = a[:, 128*k:128*(k+1)]
                    g = jnp.take_along_axis(ak, lane_grp + 4*s, axis=1)
                    ls.append(jnp.where(diag, g, 0.0).astype(BF16))
                l = jnp.concatenate(ls, axis=1)
                acc = acc + jnp.dot(l, wref[pl.ds(ch*cq, cq), :], preferred_element_type=F32)
            return acc

        q = contract_lead(jnp.broadcast_to(xn, (H, M)), qb, 'q')
        qbf = q.astype(BF16)

        accs = [jnp.zeros((H, 128), F32) for _ in range(4)]
        gidx = (lane % 4) * 32 + row
        for ch in range(nq):
            wait('uk', ch)
            o_ = lax.dot_general(qbf, ukb[pl.ds(ch*cq, cq), :], (((1,), (1,)), ((), ())), preferred_element_type=F32)
            for tt in range(tiles_per_chunk):
                t = ch * tiles_per_chunk + tt
                k, s = t // 32, t % 32
                g = jnp.take_along_axis(o_[:, tt*128:(tt+1)*128], gidx, axis=1)
                accs[k] = jnp.where(lane // 4 == s, g, accs[k])
        A = jnp.concatenate(accs, axis=1) * (D ** -0.5)
        Abf = A.astype(BF16)

        def kv_body(i, carry):
            m, l, acc = carry
            start = pl.multiple_of(i * bk, bk)
            pltpu.make_async_copy(ckv_hbm.at[pl.ds(start, bk)], cb.at[pl.ds(start, bk)], sem_c.at[i]).wait()
            @pl.when(i + W < nkv)
            def _():
                s2 = pl.multiple_of((i + W) * bk, bk)
                pltpu.make_async_copy(ckv_hbm.at[pl.ds(s2, bk)], cb.at[pl.ds(s2, bk)], sem_c.at[i + W]).start()
            for ii in range(max(0, nkv - W), nkv):
                j = base['c'] + ii + W
                if j < NP:
                    @pl.when(i == ii)
                    def _():
                        cp(j).start()
            s = lax.dot_general(Abf, cb[pl.ds(start, bk), :], (((1,), (1,)), ((), ())), preferred_element_type=F32)
            m_new = jnp.maximum(m, jnp.max(s, axis=1, keepdims=True))
            alpha = jnp.exp(m - m_new)
            p = jnp.exp(s - m_new)
            l = alpha * l + jnp.sum(p, axis=1, keepdims=True)
            acc = alpha * acc + jnp.dot(p.astype(BF16), cb[pl.ds(start, bk), :], preferred_element_type=F32)
            return m_new, l, acc
        m0 = jnp.full((H, 1), -jnp.inf, F32)
        m, l, acc = lax.fori_loop(0, nkv, kv_body, (m0, jnp.zeros((H, 1), F32), jnp.zeros((H, DC), F32)))
        ctxc = (acc / l).astype(BF16).astype(F32)

        ctx = contract_lead(ctxc, uvb, 'uv')

        heads_per = H // no
        o_acc = jnp.zeros((H, M), F32)
        for ch in range(no):
            wait('o', ch)
            l_ = jnp.concatenate([jnp.where(row == ch*heads_per + j, ctx, 0.0).astype(BF16) for j in range(heads_per)], axis=1)
            o_acc = o_acc + jnp.dot(l_, ob[pl.ds(ch*co, co), :], preferred_element_type=F32)
        hres = x + jnp.sum(o_acc, axis=0, keepdims=True).astype(BF16).astype(F32)
        hres = hres.astype(BF16).astype(F32)
        hn = _ln(hres).astype(BF16)
        hn8 = jnp.broadcast_to(hn, (16, M))

        cb1.wait()
        b1 = b1b[...].astype(F32)
        z = jnp.zeros((16, M), F32)
        acts = []
        for i, (s, n) in enumerate(f1):
            wait('w1', i)
            y = lax.dot_general(hn8, w1b[pl.ds(s, n), :], (((1,), (1,)), ((), ())), preferred_element_type=F32)
            y = y + b1[s:s+n][None, :]
            sp = jnp.log1p(jnp.exp(-jnp.abs(y))) + jnp.maximum(y, 0.0)
            acts.append((y * jnp.tanh(sp)).astype(BF16))
        act = jnp.concatenate(acts, axis=1)
        for i, (s, n) in enumerate(f2):
            wait('w2', i)
            z = z + jnp.dot(act[:, s:s+n], w2b[pl.ds(s, n), :], preferred_element_type=F32)
        o_ref[...] = (hres + z[0:1]).astype(BF16)

    @jax.jit
    def fn(A_x, A_c_kv, A_w_q, A_w_uk, A_w_uv, A_w_o, B_x, B_w1, B_b1, B_w2):
        anyspec = pl.BlockSpec(memory_space=pl.ANY)
        out = pl.pallas_call(
            kernel,
            out_shape=jax.ShapeDtypeStruct((1, M), BF16),
            in_specs=[anyspec]*9,
            out_specs=pl.BlockSpec(memory_space=pltpu.VMEM),
            scratch_shapes=[pltpu.VMEM((1, M), BF16), pltpu.VMEM((F,), BF16),
                            pltpu.VMEM((16384, 128), BF16), pltpu.VMEM((16384, 128), BF16), pltpu.VMEM((SK, DC), BF16),
                            pltpu.VMEM((16384, 128), BF16), pltpu.VMEM((4096, M), BF16), pltpu.VMEM((F, M), BF16), pltpu.VMEM((F, M), BF16),
                            pltpu.SemaphoreType.DMA((2,)), pltpu.SemaphoreType.DMA((nq,)), pltpu.SemaphoreType.DMA((nq,)), pltpu.SemaphoreType.DMA((nkv,)),
                            pltpu.SemaphoreType.DMA((nq,)), pltpu.SemaphoreType.DMA((no,)), pltpu.SemaphoreType.DMA((len(f1),)), pltpu.SemaphoreType.DMA((len(f2),))],
            compiler_params=pltpu.CompilerParams(vmem_limit_bytes=64*1024*1024),
        )(A_x.reshape(1, M), A_c_kv.reshape(SK, DC), A_w_q.reshape(16384, 128), A_w_uk.reshape(16384, 128), A_w_uv.reshape(16384, 128),
          A_w_o.reshape(4096, M), B_w1.T, B_b1, B_w2)
        return out.reshape(1, 1, M)
    return fn


_FN = build(window=3, nkv=8)


def pallas_sequential_preLN__compressed_kv_cla__dense_activation_mish__decode_kernel(
    A_x, A_c_kv, A_w_q, A_w_uk, A_w_uv, A_w_o, B_x, B_w1, B_b1, B_w2
):
    return _FN(A_x, A_c_kv, A_w_q, A_w_uk, A_w_uv, A_w_o, B_x, B_w1, B_b1, B_w2)
```

```python
import jax
import jax.numpy as jnp
import jax.experimental.pallas as pl
import jax.experimental.pallas.tpu as pltpu
from jax import lax

F32 = jnp.float32
BF16 = jnp.bfloat16

H, D, M, SK, DC, F = 32, 128, 512, 8192, 512, 1376
WROWS = M * H

NT = (((1,), (1,)), ((), ()))

N_W = 4
N_KV = 8
W_CHUNK = WROWS // N_W
KV_CHUNK = SK // N_KV
O_CHUNK = H * D // N_W
F1_CHUNKS = ((0, 512), (512, 512), (1024, 352))
F2_CHUNKS = ((0, 512), (512, 512), (1024, 256), (1280, 96))
INFLIGHT = 3


def _layernorm(v):
    mu = jnp.mean(v, axis=-1, keepdims=True)
    c = v - mu
    var = jnp.mean(c * c, axis=-1, keepdims=True)
    return c / jnp.sqrt(var + 1e-5)


def _round_bf16(v):
    return v.astype(BF16).astype(F32)


def _kernel(x_hbm, ckv_hbm, wq_hbm, wuk_hbm, wuv_hbm, wo_hbm, w1t_hbm, b1_hbm, w2_hbm,
            o_ref,
            x_buf, b1_buf, wq_buf, wuk_buf, ckv_buf, wuv_buf, wo_buf, w1_buf, w2_buf, sems):
    plan = []
    first = {}

    def add(name, src, dst, chunks=None):
        first[name] = len(plan)
        if chunks is None:
            plan.append((src, dst))
        else:
            for start, size in chunks:
                plan.append((src.at[pl.ds(start, size)], dst.at[pl.ds(start, size)]))

    w_chunks = [(i * W_CHUNK, W_CHUNK) for i in range(N_W)]
    add("wq", wq_hbm, wq_buf, w_chunks[:1])
    add("x", x_hbm, x_buf)
    add("wq_rest", wq_hbm, wq_buf, w_chunks[1:])
    add("wuk", wuk_hbm, wuk_buf, w_chunks)
    add("ckv", ckv_hbm, ckv_buf, [(i * KV_CHUNK, KV_CHUNK) for i in range(N_KV)])
    add("wuv", wuv_hbm, wuv_buf, w_chunks)
    add("wo", wo_hbm, wo_buf, [(i * O_CHUNK, O_CHUNK) for i in range(N_W)])
    add("b1", b1_hbm, b1_buf)
    add("w1", w1t_hbm, w1_buf, F1_CHUNKS)
    add("w2", w2_hbm, w2_buf, F2_CHUNKS)

    def copy(j):
        return pltpu.make_async_copy(plan[j][0], plan[j][1], sems.at[j % INFLIGHT])

    def wait(name, i=0):
        j = first[name] + i
        copy(j).wait()
        if j + INFLIGHT < len(plan):
            copy(j + INFLIGHT).start()

    for j in range(INFLIGHT):
        copy(j).start()

    row = lax.broadcasted_iota(jnp.int32, (H, 128), 0)
    lane = lax.broadcasted_iota(jnp.int32, (H, 128), 1)
    on_diag = (lane % H) == row
    tiles = W_CHUNK // 128

    def contract_lead(a, w_buf, waits):
        acc = jnp.zeros((H, D), F32)
        for ch in range(N_W):
            waits(ch)
            blocks = []
            for tt in range(tiles):
                k, s = divmod(ch * tiles + tt, 32)
                g = jnp.take_along_axis(a[:, 128 * k:128 * (k + 1)], lane // H + 4 * s, axis=1)
                blocks.append(jnp.where(on_diag, g, 0.0).astype(BF16))
            lhs = jnp.concatenate(blocks, axis=1)
            acc = acc + jnp.dot(lhs, w_buf[pl.ds(ch * W_CHUNK, W_CHUNK), :],
                                preferred_element_type=F32)
        return acc

    wait("x")
    x = x_buf[...].astype(F32)
    xn = _round_bf16(_layernorm(x))
    q = contract_lead(jnp.broadcast_to(xn, (H, M)), wq_buf,
                      lambda ch: wait("wq") if ch == 0 else wait("wq_rest", ch - 1))
    q = q.astype(BF16)

    a_tiles = [jnp.zeros((H, 128), F32) for _ in range(DC // 128)]
    diag_idx = (lane % 4) * H + row
    for ch in range(N_W):
        wait("wuk", ch)
        full = lax.dot_general(q, wuk_buf[pl.ds(ch * W_CHUNK, W_CHUNK), :], NT,
                               preferred_element_type=F32)
        for tt in range(tiles):
            k, s = divmod(ch * tiles + tt, 32)
            g = jnp.take_along_axis(full[:, tt * 128:(tt + 1) * 128], diag_idx, axis=1)
            a_tiles[k] = jnp.where(lane // 4 == s, g, a_tiles[k])
    a = jnp.concatenate(a_tiles, axis=1) * (D ** -0.5)
    a_hi = a.astype(BF16)
    a_lo = (a - a_hi.astype(F32)).astype(BF16)
    a2 = jnp.concatenate([a_hi, a_lo], axis=0)

    m = jnp.full((H, 1), -jnp.inf, F32)
    l = jnp.zeros((H, 1), F32)
    acc = jnp.zeros((H, DC), F32)
    for i in range(N_KV):
        wait("ckv", i)
        s2 = lax.dot_general(a2, ckv_buf[pl.ds(i * KV_CHUNK, KV_CHUNK), :], NT,
                             preferred_element_type=F32)
        s = s2[:H] + s2[H:]
        m_new = jnp.maximum(m, jnp.max(s, axis=1, keepdims=True))
        alpha = jnp.exp(m - m_new)
        p = jnp.exp(s - m_new)
        l = alpha * l + jnp.sum(p, axis=1, keepdims=True)
        acc = alpha * acc + jnp.dot(p.astype(BF16), ckv_buf[pl.ds(i * KV_CHUNK, KV_CHUNK), :],
                                    preferred_element_type=F32)
        m = m_new
    ctx_c = _round_bf16(acc / l)

    ctx = contract_lead(ctx_c, wuv_buf, lambda ch: wait("wuv", ch))

    heads = O_CHUNK // D
    o_acc = jnp.zeros((H, M), F32)
    for ch in range(N_W):
        wait("wo", ch)
        lhs = jnp.concatenate(
            [jnp.where(row == ch * heads + j, ctx, 0.0).astype(BF16) for j in range(heads)], axis=1)
        o_acc = o_acc + jnp.dot(lhs, wo_buf[pl.ds(ch * O_CHUNK, O_CHUNK), :],
                                preferred_element_type=F32)
    attn = _round_bf16(jnp.sum(o_acc, axis=0, keepdims=True))
    h = _round_bf16(x + attn)

    hn = jnp.broadcast_to(_layernorm(h).astype(BF16), (16, M))
    wait("b1")
    b1 = b1_buf[...].astype(F32)
    acts = []
    for i, (start, size) in enumerate(F1_CHUNKS):
        wait("w1", i)
        y = lax.dot_general(hn, w1_buf[pl.ds(start, size), :], NT, preferred_element_type=F32)
        y = y + b1[start:start + size][None, :]
        softplus = jnp.log1p(jnp.exp(-jnp.abs(y))) + jnp.maximum(y, 0.0)
        acts.append((y * jnp.tanh(softplus)).astype(BF16))
    act = jnp.concatenate(acts, axis=1)

    z = jnp.zeros((16, M), F32)
    for i, (start, size) in enumerate(F2_CHUNKS):
        wait("w2", i)
        z = z + jnp.dot(act[:, start:start + size], w2_buf[pl.ds(start, size), :],
                        preferred_element_type=F32)
    o_ref[...] = (h + z[0:1]).astype(BF16)


@jax.jit
def pallas_sequential_preLN__compressed_kv_cla__dense_activation_mish__decode_kernel(
    A_x: jax.Array,
    A_c_kv: jax.Array,
    A_w_q: jax.Array,
    A_w_uk: jax.Array,
    A_w_uv: jax.Array,
    A_w_o: jax.Array,
    B_x: jax.Array,
    B_w1: jax.Array,
    B_b1: jax.Array,
    B_w2: jax.Array,
):
    del B_x
    out = pl.pallas_call(
        _kernel,
        out_shape=jax.ShapeDtypeStruct((1, M), BF16),
        in_specs=[pl.BlockSpec(memory_space=pl.ANY)] * 9,
        out_specs=pl.BlockSpec(memory_space=pltpu.VMEM),
        scratch_shapes=[
            pltpu.VMEM((1, M), BF16),
            pltpu.VMEM((F,), BF16),
            pltpu.VMEM((WROWS, D), BF16),
            pltpu.VMEM((WROWS, D), BF16),
            pltpu.VMEM((SK, DC), BF16),
            pltpu.VMEM((WROWS, D), BF16),
            pltpu.VMEM((H * D, M), BF16),
            pltpu.VMEM((F, M), BF16),
            pltpu.VMEM((F, M), BF16),
            pltpu.SemaphoreType.DMA((INFLIGHT,)),
        ],
        compiler_params=pltpu.CompilerParams(vmem_limit_bytes=64 * 1024 * 1024),
    )(
        A_x.reshape(1, M),
        A_c_kv.reshape(SK, DC),
        A_w_q.reshape(WROWS, D),
        A_w_uk.reshape(WROWS, D),
        A_w_uv.reshape(WROWS, D),
        A_w_o.reshape(H * D, M),
        B_w1.T,
        B_b1,
        B_w2,
    )
    return out.reshape(1, 1, M)
```
